```python
import os as _os
_os.environ.setdefault("JAX_PLATFORMS", "cpu")
import jax
import jax.numpy as jnp

def _softmax(x, axis=-1):
    return jax.nn.softmax(x, axis=axis)
def _gelu(x):
    return jax.nn.gelu(x, approximate=True)
def _silu(x):
    return jax.nn.silu(x)
def _sigmoid(x):
    return jax.nn.sigmoid(x)
def _layernorm(x, axis=-1, eps=1e-5):
    m = jnp.mean(x, axis=axis, keepdims=True)
    v = jnp.var(x, axis=axis, keepdims=True)
    return (x - m) / jnp.sqrt(v + eps)
def _scatter_add(tgt, idx, src, axis=0):
    return tgt.at[idx].add(src)
def _segment_sum(src, seg, n):
    return jax.ops.segment_sum(src, seg, n)
class _Rng:
    def __init__(self, key):
        self._k = key
    def _next(self):
        self._k, sub = jax.random.split(self._k)
        return sub
    def normal(self, shape):
        return jax.random.normal(self._next(), shape, dtype=jnp.bfloat16)
    def randint(self, lo, hi, shape):
        return jax.random.randint(self._next(), shape, lo, hi, dtype=jnp.int32)
    def uniform(self, shape, lo=0.0, hi=1.0):
        return jax.random.uniform(self._next(), shape, jnp.bfloat16, lo, hi)
    def permutation(self, n):
        return jax.random.permutation(self._next(), n)


kernel_name = 'standalone__gqa_block_cached__sampling'

def setup_inputs():
    _rng = _Rng(jax.random.key(int.from_bytes(__import__("os").urandom(4), "little")))
    _w = (lambda a: (lambda t: t.astype(jnp.bfloat16) if jnp.issubdtype(t.dtype, jnp.floating) else t)(jnp.asarray(a)))
    B, Sq, D = 32, 16, 1024
    Hq, Hkv, Sk, Dh = 32, 4, 2048, 128
    assert Hq % Hkv == 0, (Hq, Hkv)
    return {
        "x": _w((lambda *s: _rng.normal(s) * 0.8)(B, Sq, D)),
        "k_cache": _w((lambda *s: _rng.normal(s) * 0.8)(B, Hkv, Sk, Dh)),
        "v_cache": _w((lambda *s: _rng.normal(s) * 0.05)(B, Hkv, Sk, Dh)),
        "wq": _w((lambda *s: _rng.normal(s) * 0.8)(D, Hq * Dh) * (D ** -0.5)),
        "wo": _w((lambda *s: _rng.normal(s) * 0.05)(Hq * Dh, D) * ((Hq * Dh) ** -0.5)),
    }

def reference(x, k_cache, v_cache, wq, wo):
    B, Sq, D = x.shape
    Hq, Dh = 32, 128
    Hkv = k_cache.shape[1]
    rep = Hq // Hkv
    q = (lambda x, *d: x.transpose(*d))((x @ wq).reshape(B, Sq, Hq, Dh), 0, 2, 1, 3)
    k = jnp.repeat(k_cache, rep, axis=1)
    v = jnp.repeat(v_cache, rep, axis=1)
    scores = jnp.einsum("bhqd,bhkd->bhqk", q, k) * (Dh ** -0.5)
    p = _softmax(scores, axis=-1)
    o = jnp.einsum("bhqk,bhkd->bhqd", p, v)
    return (lambda x, *d: x.transpose(*d))(o, 0, 2, 1, 3).reshape(B, Sq, Hq * Dh) @ wo
```

```python
import math
import jax
import jax.numpy as jnp
import jax.experimental.pallas as pl
import jax.experimental.pallas.tpu as pltpu

NT = (((1,), (1,)), ((), ()))

def make(NBUF=8, scopes=False):
    B, Sq, D = 32, 16, 1024
    Hq, Hkv, Sk, Dh = 32, 4, 2048, 128
    REP = Hq // Hkv
    GW = REP * Dh
    ROWS = B * Sq
    BB = 8
    CH = BB * Sq
    NCH = ROWS // CH
    NUNITS = B * Hkv
    QSCALE = (Dh ** -0.5) * math.log2(math.e)
    import contextlib
    ns = (lambda n: jax.named_scope(n)) if scopes else (lambda n: contextlib.nullcontext())

    def kernel(x_hbm, k_hbm, v_hbm, wq_hbm, wo_hbm, out_hbm,
               x_buf, wq_buf, wo_buf, k_buf, v_buf, q_s, o_s, acc, out_buf,
               x_sem, wq_sem, wo_sem, k_sem, v_sem, out_sem):
        def x_cp():
            return pltpu.make_async_copy(x_hbm, x_buf, x_sem.at[0])
        def wq_cp(h):
            return pltpu.make_async_copy(wq_hbm.at[:, pl.ds(pl.multiple_of(h * GW, GW), GW)], wq_buf.at[h], wq_sem.at[h])
        def wo_cp(h):
            return pltpu.make_async_copy(wo_hbm.at[pl.ds(pl.multiple_of(h * GW, GW), GW), :], wo_buf.at[h], wo_sem.at[h])
        def k_cp(u, slot):
            return pltpu.make_async_copy(k_hbm.at[u % B, u // B], k_buf.at[slot], k_sem.at[slot])
        def v_cp(u, slot):
            return pltpu.make_async_copy(v_hbm.at[u % B, u // B], v_buf.at[slot], v_sem.at[slot])
        def out_cp(c):
            rows = pl.ds(pl.multiple_of(c * CH, CH), CH)
            return pltpu.make_async_copy(out_buf.at[rows, :], out_hbm.at[rows, :], out_sem.at[c])

        def issue_unit_static(u):
            if u % B == 0:
                wq_cp(u // B).start()
            k_cp(u, u % NBUF).start()
            v_cp(u, u % NBUF).start()
            if u % B == BB - 1:
                wo_cp(u // B).start()

        def issue_unit(u, slot):
            @pl.when(u % B == 0)
            def _():
                wq_cp(u // B).start()
            k_cp(u, slot).start()
            v_cp(u, slot).start()
            @pl.when(u % B == BB - 1)
            def _():
                wo_cp(u // B).start()

        with ns("prologue"):
            x_cp().start()
            for u in range(NBUF):
                issue_unit_static(u)
            acc[...] = jnp.zeros_like(acc)
            x_cp().wait()

        def super_unit(s, _):
            h = s // NCH
            c = s % NCH
            rows = pl.ds(pl.multiple_of(c * CH, CH), CH)
            with ns("wait_wq"):
                @pl.when(c == 0)
                def _():
                    wq_cp(h).wait()
            with ns("qproj"):
                q = jnp.dot(x_buf[rows, :], wq_buf[h], preferred_element_type=jnp.float32)
                q_s[...] = (q * QSCALE).astype(jnp.bfloat16)

            def unit(i, _):
                u = s * BB + i
                slot = u % NBUF
                with ns("wait_kv"):
                    k_cp(u, slot).wait()
                    v_cp(u, slot).wait()
                with ns("attn"):
                    r = pl.ds(pl.multiple_of(i * Sq, Sq), Sq)
                    qb = q_s[r, :]
                    qq = jnp.concatenate([qb[:, j * Dh:(j + 1) * Dh] for j in range(REP)], axis=0)
                    sc = jax.lax.dot_general(qq, k_buf[slot], NT, preferred_element_type=jnp.float32)
                    m = jnp.max(sc, axis=1, keepdims=True)
                    p = jnp.exp2(sc - m)
                    l = jnp.sum(p, axis=1, keepdims=True)
                    o = jnp.dot(p.astype(jnp.bfloat16), v_buf[slot], preferred_element_type=jnp.float32)
                    o = (o / l).astype(jnp.bfloat16)
                    for j in range(REP):
                        o_s[r, j * Dh:(j + 1) * Dh] = o[j * Sq:(j + 1) * Sq, :]
                with ns("issue"):
                    @pl.when(u + NBUF < NUNITS)
                    def _():
                        issue_unit(u + NBUF, slot)
                return 0
            jax.lax.fori_loop(0, BB, unit, 0)

            with ns("wait_wo"):
                @pl.when(c == 0)
                def _():
                    wo_cp(h).wait()
            with ns("oproj"):
                y = jnp.dot(o_s[...], wo_buf[h], preferred_element_type=jnp.float32)
                acc[rows, :] += y

                @pl.when(h == Hkv - 1)
                def _():
                    out_buf[rows, :] = acc[rows, :].astype(jnp.bfloat16)
                    out_cp(c).start()
            return 0
        jax.lax.fori_loop(0, Hkv * NCH, super_unit, 0)
        with ns("final"):
            for c in range(NCH):
                out_cp(c).wait()

    @jax.jit
    def f(x, k_cache, v_cache, wq, wo):
        x2 = x.reshape(ROWS, D)
        out = pl.pallas_call(
            kernel,
            out_shape=jax.ShapeDtypeStruct((ROWS, D), jnp.bfloat16),
            in_specs=[pl.BlockSpec(memory_space=pl.ANY)] * 5,
            out_specs=pl.BlockSpec(memory_space=pl.ANY),
            scratch_shapes=[
                pltpu.VMEM((ROWS, D), jnp.bfloat16),
                pltpu.VMEM((Hkv, D, GW), jnp.bfloat16),
                pltpu.VMEM((Hkv, GW, D), jnp.bfloat16),
                pltpu.VMEM((NBUF, Sk, Dh), jnp.bfloat16),
                pltpu.VMEM((NBUF, Sk, Dh), jnp.bfloat16),
                pltpu.VMEM((CH, GW), jnp.bfloat16),
                pltpu.VMEM((CH, GW), jnp.bfloat16),
                pltpu.VMEM((ROWS, D), jnp.float32),
                pltpu.VMEM((ROWS, D), jnp.bfloat16),
                pltpu.SemaphoreType.DMA((1,)),
                pltpu.SemaphoreType.DMA((Hkv,)),
                pltpu.SemaphoreType.DMA((Hkv,)),
                pltpu.SemaphoreType.DMA((NBUF,)),
                pltpu.SemaphoreType.DMA((NBUF,)),
                pltpu.SemaphoreType.DMA((NCH,)),
            ],
            compiler_params=pltpu.CompilerParams(vmem_limit_bytes=100 * 1024 * 1024),
        )(x2, k_cache, v_cache, wq, wo)
        return out.reshape(B, Sq, D)
    return f

pallas_standalone__gqa_block_cached__sampling_kernel = make(8)
```

```python
import math
import contextlib
import jax
import jax.numpy as jnp
import jax.experimental.pallas as pl
import jax.experimental.pallas.tpu as pltpu

NT = (((1,), (1,)), ((), ()))

def make(LK=3, LV=10, scopes=False, nsplit=2, tail=(64, 64), NL=1, qsplit=2, xorder=False,
         pk=0, pv_=1, pwq=0, pwo=1, kswitch=128, wq_at=15, wo_at="q", px=0):
    B, Sq, D = 32, 16, 1024
    Hq, Hkv, Sk, Dh = 32, 4, 2048, 128
    REP = Hq // Hkv
    GW = REP * Dh
    ROWS = B * Sq
    CH = 128
    NCH = ROWS // CH
    OCH = 128
    NUNITS = B * Hkv
    QSCALE = (Dh ** -0.5) * math.log2(math.e)
    NK, NV = LK, LV
    def ns(n):
        if scopes is True or (scopes == 2 and n.startswith("P_")):
            return jax.named_scope(n)
        return contextlib.nullcontext()
    TAILROWS = sum(tail)
    TAILU = TAILROWS // Sq
    OB = OCH // Sq
    assert TAILROWS % OCH == 0
    LASTN = tail[-1]
    EARLY = ROWS - LASTN
    NMAIN = NUNITS - NL
    assert NL <= LK and NL <= LV

    def kernel(x_hbm, k_hbm, v_hbm, wq_hbm, wo_hbm, out_hbm,
               x_buf, wq_buf, wo_buf, k_buf, v_buf, q_s, o_s, acc, out_buf,
               x_sem, wq_sem, wo_sem, k_sem, v_sem, out_sem):
        def x_cp():
            return pltpu.make_async_copy(x_hbm, x_buf, x_sem.at[0])
        def wq_cp(h):
            return pltpu.make_async_copy(wq_hbm.at[:, pl.ds(pl.multiple_of(h * GW, GW), GW)], wq_buf.at[h], wq_sem.at[h])
        def wo_cp(h):
            return pltpu.make_async_copy(wo_hbm.at[pl.ds(pl.multiple_of(h * GW, GW), GW), :], wo_buf.at[h], wo_sem.at[h])
        def k_cp(u):
            return pltpu.make_async_copy(k_hbm.at[u % B, u // B], k_buf.at[u % NK], k_sem.at[u % NK])
        def v_cp(u):
            return pltpu.make_async_copy(v_hbm.at[u % B, u // B], v_buf.at[u % NV], v_sem.at[u % NV])
        def out_cp(r0, n, si):
            rows = pl.ds(r0, n)
            return pltpu.make_async_copy(out_buf.at[rows, :], out_hbm.at[rows, :], out_sem.at[si])

        def issue_k(n):
            if pv_ != pk and kswitch < NUNITS:
                @pl.when(n < kswitch)
                def _():
                    k_cp(n).start(priority=pk)
                @pl.when(jnp.logical_and(n >= kswitch, n < NUNITS))
                def _():
                    k_cp(n).start(priority=pv_)
            else:
                @pl.when(n < NUNITS)
                def _():
                    k_cp(n).start(priority=pk)
        def issue_v(n):
            @pl.when(n < NUNITS)
            def _():
                v_cp(n).start(priority=pv_)

        with ns("P_prologue"):
            x_cp().start(priority=px)
            wq_cp(0).start(priority=px)
            def first(n, _):
                @pl.when(n < LK)
                def _():
                    k_cp(n).start(priority=pk)
                @pl.when(n < LV)
                def _():
                    v_cp(n).start(priority=pv_)
                return 0
            jax.lax.fori_loop(0, max(LK, LV), first, 0)
            acc[...] = jnp.zeros_like(acc)
            x_cp().wait()

        def sm(sc):
            m = jnp.max(sc, axis=1, keepdims=True)
            p = jnp.exp2(sc - m)
            l = jnp.sum(p, axis=1, keepdims=True)
            return p.astype(jnp.bfloat16), l

        def qk(u, ns_):
            JR = REP // ns_
            r = pl.ds(pl.multiple_of((u % B) * Sq, Sq), Sq)
            qb = q_s[r, :]
            kk = k_buf[u % NK]
            scs = []
            for t in range(ns_):
                qq = jnp.concatenate([qb[:, j * Dh:(j + 1) * Dh] for j in range(t * JR, (t + 1) * JR)], axis=0)
                scs.append(jax.lax.dot_general(qq, kk, NT, preferred_element_type=jnp.float32))
            return scs
        def pvf(u, t, ns_, p, l):
            JR = REP // ns_
            r = pl.ds(pl.multiple_of((u % B) * Sq, Sq), Sq)
            o = jnp.dot(p, v_buf[u % NV], preferred_element_type=jnp.float32)
            o = (o * (1.0 / l)).astype(jnp.bfloat16)
            for jj in range(JR):
                j = t * JR + jj
                o_s[r, j * Dh:(j + 1) * Dh] = o[jj * Sq:(jj + 1) * Sq, :]
        def attention(u):
            scs = qk(u, nsplit)
            for t in range(nsplit):
                p, l = sm(scs[t])
                pvf(u, t, nsplit, p, l)

        def oproj_final(r0, n):
            y = jnp.dot(o_s[pl.ds(r0, n), :], wo_buf[Hkv - 1], preferred_element_type=jnp.float32)
            out_buf[pl.ds(r0, n), :] = (acc[pl.ds(r0, n), :] + y).astype(jnp.bfloat16)

        def step(u, _):
            h = u // B
            b = u % B

            @pl.when(b == 0)
            def _():
                with ns("wait_wq"):
                    wq_cp(h).wait()
                with ns("qproj"):
                    if wo_at == "q":
                        wo_cp(h).start(priority=pwo)
                    def qp(c, _):
                        rows = pl.ds(pl.multiple_of(c * CH, CH), CH)
                        q = jnp.dot(x_buf[rows, :], wq_buf[h], preferred_element_type=jnp.float32)
                        q_s[rows, :] = (q * QSCALE).astype(jnp.bfloat16)
                        return 0
                    jax.lax.fori_loop(0, NCH, qp, 0)

            with ns("wait_k"):
                k_cp(u).wait()
            with ns("wait_v"):
                v_cp(u).wait()
            with ns("attn"):
                attention(u)
            with ns("issue"):
                issue_k(u + LK)
                issue_v(u + LV)
                if wo_at != "q":
                    @pl.when(b == wo_at)
                    def _():
                        wo_cp(h).start(priority=pwo)
                @pl.when(jnp.logical_and(b == wq_at, h < Hkv - 1))
                def _():
                    wq_cp(h + 1).start(priority=pwq)

            @pl.when(jnp.logical_and(b % OB == OB - 1, u < NUNITS - TAILU))
            def _():
                rows = pl.ds(pl.multiple_of((b // OB) * OCH, OCH), OCH)
                with ns("wait_wo"):
                    @pl.when(b == OB - 1)
                    def _():
                        wo_cp(h).wait()
                with ns("oproj"):
                    y = jnp.dot(o_s[rows, :], wo_buf[h], preferred_element_type=jnp.float32)
                    @pl.when(h < Hkv - 1)
                    def _():
                        acc[rows, :] += y
                    @pl.when(h == Hkv - 1)
                    def _():
                        out_buf[rows, :] = (acc[rows, :] + y).astype(jnp.bfloat16)
            off = ROWS - TAILROWS
            for ti, n in enumerate(tail[:-1]):
                last_u = (Hkv - 1) * B + (off + n) // Sq - 1
                def piece(off=off, n=n, ti=ti):
                    with ns(f"oproj_t{ti}"):
                        oproj_final(off, n)
                assert last_u < NMAIN
                pl.when(u == last_u)(piece)
                off += n
            return 0
        with ns("P_mainloop"):
            jax.lax.fori_loop(0, NMAIN, step, 0)

        pend = {}
        def qpart(u):
            with ns(f"P_wait_k{u}"):
                k_cp(u).wait()
            with ns(f"P_q{u}"):
                pend[u] = [sm(sc) for sc in qk(u, qsplit)]
        def ppart(u):
            with ns(f"P_wait_v{u}"):
                v_cp(u).wait()
                if u == NUNITS - 1:
                    out_cp(0, EARLY, 0).start()
            with ns(f"P_p{u}"):
                for t in range(qsplit):
                    pvf(u, t, qsplit, *pend[u][t])
        if xorder:
            for u in range(NMAIN, NUNITS): qpart(u)
            for u in range(NMAIN, NUNITS): ppart(u)
        else:
            for u in range(NMAIN, NUNITS):
                qpart(u); ppart(u)
        with ns("P_oproj_last"):
            oproj_final(EARLY, LASTN)
            out_cp(EARLY, LASTN, 1).start()
        with ns("P_final"):
            out_cp(0, EARLY, 0).wait()
            out_cp(EARLY, LASTN, 1).wait()

    @jax.jit
    def f(x, k_cache, v_cache, wq, wo):
        x2 = x.reshape(ROWS, D)
        out = pl.pallas_call(
            kernel,
            out_shape=jax.ShapeDtypeStruct((ROWS, D), jnp.bfloat16),
            in_specs=[pl.BlockSpec(memory_space=pl.ANY)] * 5,
            out_specs=pl.BlockSpec(memory_space=pl.ANY),
            scratch_shapes=[
                pltpu.VMEM((ROWS, D), jnp.bfloat16),
                pltpu.VMEM((Hkv, D, GW), jnp.bfloat16),
                pltpu.VMEM((Hkv, GW, D), jnp.bfloat16),
                pltpu.VMEM((NK, Sk, Dh), jnp.bfloat16),
                pltpu.VMEM((NV, Sk, Dh), jnp.bfloat16),
                pltpu.VMEM((ROWS, GW), jnp.bfloat16),
                pltpu.VMEM((ROWS, GW), jnp.bfloat16),
                pltpu.VMEM((ROWS, D), jnp.float32),
                pltpu.VMEM((ROWS, D), jnp.bfloat16),
                pltpu.SemaphoreType.DMA((1,)),
                pltpu.SemaphoreType.DMA((Hkv,)),
                pltpu.SemaphoreType.DMA((Hkv,)),
                pltpu.SemaphoreType.DMA((NK,)),
                pltpu.SemaphoreType.DMA((NV,)),
                pltpu.SemaphoreType.DMA((2,)),
            ],
            compiler_params=pltpu.CompilerParams(vmem_limit_bytes=100 * 1024 * 1024),
        )(x2, k_cache, v_cache, wq, wo)
        return out.reshape(B, Sq, D)
    return f


pallas_standalone__gqa_block_cached__sampling_kernel = make(LK=2, LV=10, pwo=0, pwq=1)
```

```python
import math
import contextlib
import jax
import jax.numpy as jnp
import jax.experimental.pallas as pl
import jax.experimental.pallas.tpu as pltpu

NT = (((1,), (1,)), ((), ()))

def make(LP=2, LD=10, QA=3, scopes=False, anchors=None, order="aqo", tailrows=64, nobounds=False,
         t1order="VVVqVVVoVVVV", anchor=True, wanch=("sA7", "pB7"), wprio=0):
    B, Sq, D = 32, 16, 1024
    Hq, Hkv, Sk, Dh = 32, 4, 2048, 128
    REP = Hq // Hkv
    GW = REP * Dh
    ROWS = B * Sq
    CH = 128
    NCH = ROWS // CH
    OB = CH // Sq
    NUNITS = B * Hkv
    NS = NUNITS // OB
    QSCALE = (Dh ** -0.5) * math.log2(math.e)
    NQ, NK, NV = 4, 4, 16
    assert QA == 3 and LP < NK and LD <= NV
    def ns(n):
        if scopes is True or (scopes == 2 and n.startswith("P_")):
            return jax.named_scope(n)
        return contextlib.nullcontext()
    LASTN = tailrows
    EARLY = ROWS - LASTN
    JR = REP // 2
    if anchors is None:
        anchors = ["top", "sA15", "sB7", "sB15", "oA", "oB", "q", "y"]
    G = len(anchors)
    PR = Sk // G
    assert PR % Sq == 0 and t1order.count("V") == LD

    def kernel(x_hbm, k_hbm, v_hbm, wq_hbm, wo_hbm, out_hbm,
               x_buf, wq_buf, wo_buf, k_buf, v_buf, q_s, o_s, acc, out_buf,
               x_sem, wq_sem, wo_sem, k_sem, v_sem, out_sem):
        def x_cp():
            return pltpu.make_async_copy(x_hbm, x_buf, x_sem.at[0])
        def wq_cp(h):
            return pltpu.make_async_copy(wq_hbm.at[:, pl.ds(pl.multiple_of(h * GW, GW), GW)], wq_buf.at[h], wq_sem.at[h])
        def wo_cp(h):
            return pltpu.make_async_copy(wo_hbm.at[pl.ds(pl.multiple_of(h * GW, GW), GW), :], wo_buf.at[h], wo_sem.at[h])
        WR = 32
        def wq_piece(h, j):
            r = pl.ds(pl.multiple_of(j * WR, WR), WR)
            return pltpu.make_async_copy(wq_hbm.at[r, pl.ds(pl.multiple_of(h * GW, GW), GW)], wq_buf.at[h, r], wq_sem.at[h])
        def wo_piece(h, j):
            return pltpu.make_async_copy(wo_hbm.at[pl.ds(pl.multiple_of(h * GW + j * WR, WR), WR), :], wo_buf.at[h, pl.ds(pl.multiple_of(j * WR, WR), WR)], wo_sem.at[h])
        def k_cp(u, g):
            r = pl.ds(g * PR, PR)
            return pltpu.make_async_copy(k_hbm.at[u & (B - 1), u >> 5, r], k_buf.at[u & (NK - 1), r], k_sem.at[u & (NK - 1), g])
        def v_cp(u):
            return pltpu.make_async_copy(v_hbm.at[u & (B - 1), u >> 5], v_buf.at[u & (NV - 1)], v_sem.at[u & (NV - 1)])
        def out_cp(r0, n, si):
            rows = pl.ds(r0, n)
            return pltpu.make_async_copy(out_buf.at[rows, :], out_hbm.at[rows, :], out_sem.at[si])

        def chunk_rows(s):
            return pl.ds(pl.multiple_of((s & (NCH - 1)) * CH, CH), CH)
        def col(i):
            return pl.ds(pl.multiple_of(i * Dh, Dh), Dh)

        def qpiece(s, i):
            q = jnp.dot(x_buf[chunk_rows(s), :], wq_buf[s >> 2, :, col(i)], preferred_element_type=jnp.float32)
            q = (q * QSCALE).astype(jnp.bfloat16)
            q_s[s & (NQ - 1), i] = q
            return q
        def opiece(s, i):
            rows = chunk_rows(s)
            lhs = jnp.concatenate([o_s[s & 1, j] for j in range(REP)], axis=1)
            y = jnp.dot(lhs, wo_buf[s >> 2, :, col(i)], preferred_element_type=jnp.float32)
            a = acc[rows, col(i)] + y
            acc[rows, col(i)] = a
            out_buf[rows, col(i)] = a.astype(jnp.bfloat16)
            return y
        def oproj_tail(r0, n):
            loc = r0 % CH
            lhs = jnp.concatenate([o_s[(NS - 1) & 1, j, pl.ds(loc, n), :] for j in range(REP)], axis=1)
            y = jnp.dot(lhs, wo_buf[Hkv - 1], preferred_element_type=jnp.float32)
            out_buf[pl.ds(r0, n), :] = (acc[pl.ds(r0, n), :] + y).astype(jnp.bfloat16)

        def sm(sc):
            m = jnp.max(sc, axis=1, keepdims=True)
            p = jnp.exp2(sc - m)
            l = jnp.sum(p, axis=1, keepdims=True)
            return p.astype(jnp.bfloat16), l
        def qk(u):
            s = u >> 3
            r = pl.ds(pl.multiple_of((u & (OB - 1)) * Sq, Sq), Sq)
            kk = k_buf[u & (NK - 1)]
            scs = []
            for t in range(2):
                qq = jnp.concatenate([q_s[s & (NQ - 1), j, r, :] for j in range(t * JR, (t + 1) * JR)], axis=0)
                scs.append(jax.lax.dot_general(qq, kk, NT, preferred_element_type=jnp.float32))
            return scs
        def pvf(u, t, p, l):
            s = u >> 3
            r = pl.ds(pl.multiple_of((u & (OB - 1)) * Sq, Sq), Sq)
            o = jnp.dot(p, v_buf[u & (NV - 1)], preferred_element_type=jnp.float32)
            ob = (o * (1.0 / l)).astype(jnp.bfloat16)
            for jj in range(JR):
                o_s[s & 1, t * JR + jj, r, :] = ob[jj * Sq:(jj + 1) * Sq, :]
            return ob

        def unit(u, do_q, do_o, do_k, do_v, do_w):
            s = u >> 3
            i = u & (OB - 1)
            n = u + LP
            done = set()
            def request(name, val=None):
                if not do_k or name not in anchors:
                    return
                g = anchors.index(name)
                done.add(name)
                if val is not None and anchor:
                    k_buf[n & (NK - 1), pl.ds(g * PR, Sq), :] = val[:Sq, :Dh].astype(jnp.bfloat16)
                k_cp(n, g).start(priority=0)
            def wrequest(name, val):
                if not do_w:
                    return
                g = u >> 5
                j = u & (B - 1)
                if name == wanch[0]:
                    wo_buf[Hkv, pl.ds(0, Sq), pl.ds(0, Dh)] = val[:Sq, :Dh].astype(jnp.bfloat16)
                    pl.when(g < Hkv - 1)(lambda: wo_piece(g + 1, j).start(priority=wprio))
                if name == wanch[1]:
                    wq_buf[Hkv, pl.ds(0, Sq), pl.ds(0, Dh)] = val[:Sq, :Dh].astype(jnp.bfloat16)
                    pl.when(g < Hkv - 2)(lambda: wq_piece(g + 2, j).start(priority=wprio))
            request("top")
            def part_o():
                request("y", opiece(s - 1, i) if do_o else None)
            def part_q():
                request("q", qpiece(s + QA, i) if do_q else None)
            def part_a():
                scs = qk(u)
                wrequest("sA7", scs[0][:, 7 * Dh:]); wrequest("sA15", scs[0][:, 15 * Dh:]); wrequest("sB7", scs[1][:, 7 * Dh:])
                request("sA7", scs[0][:, 7 * Dh:]); request("sA15", scs[0][:, 15 * Dh:])
                request("sB7", scs[1][:, 7 * Dh:]); request("sB15", scs[1][:, 15 * Dh:])
                pls = [sm(sc) for sc in scs]
                wrequest("pA7", pls[0][0][:, 7 * Dh:]); wrequest("pA15", pls[0][0][:, 15 * Dh:]); wrequest("pB7", pls[1][0][:, 7 * Dh:]); wrequest("pB15", pls[1][0][:, 15 * Dh:])
                request("pA7", pls[0][0][:, 7 * Dh:]); request("pA15", pls[0][0][:, 15 * Dh:])
                request("pB7", pls[1][0][:, 7 * Dh:]); request("pB15", pls[1][0][:, 15 * Dh:])
                request("oA", pvf(u, 0, *pls[0]))
                request("oB", pvf(u, 1, *pls[1]))
            for ch in order:
                {"a": part_a, "o": part_o, "q": part_q}[ch]()
            assert not do_k or done == set(anchors), (done, anchors)
            if do_v:
                v_cp(u + LD).start(priority=1)

        def weights_event(u):
            g = u >> 5
            with ns("wait_w"):
                wo_cp(g).wait()
                @pl.when(g < Hkv - 1)
                def _():
                    wq_cp(g + 1).wait()

        def make_step(do_q, do_o, do_k=True, do_v=True, events=True, tail=False, do_w=False):
            def step(u, _):
                if events:
                    pl.when((u & (B - 1)) == OB)(lambda: weights_event(u))
                with ns("wait_k"):
                    for g in range(G):
                        k_cp(u, g).wait()
                with ns("wait_v"):
                    v_cp(u).wait()
                with ns("attn"):
                    unit(u, do_q, do_o, do_k, do_v, do_w)
                if tail:
                    @pl.when(u == NUNITS - LASTN // Sq - 1)
                    def _():
                        with ns("oproj_t0"):
                            oproj_tail(ROWS - CH, CH - LASTN)
                return 0
            return step

        with ns("P_prologue"):
            x_cp().start()
            wq_cp(0).start()
            def first_k(n, _):
                for g in range(G):
                    k_cp(n, g).start(priority=0)
                return 0
            jax.lax.fori_loop(0, LP, first_k, 0)
            def first_t1(j, _):
                nv = 0
                for jj, ch in enumerate(t1order):
                    if ch == "V":
                        pl.when(j == jj)(lambda nv=nv: v_cp(nv).start(priority=1))
                        nv += 1
                    elif ch == "q":
                        pl.when(j == jj)(lambda: wq_cp(1).start(priority=1))
                    else:
                        pl.when(j == jj)(lambda: wo_cp(0).start(priority=1))
                return 0
            jax.lax.fori_loop(0, len(t1order), first_t1, 0)
            acc[...] = jnp.zeros_like(acc)
            x_cp().wait()
            wq_cp(0).wait()
        with ns("P_qproj0"):
            def q0(t, _):
                s = t >> 1
                q = jnp.dot(x_buf[chunk_rows(s), :], wq_buf[0, :, pl.ds(pl.multiple_of((t & 1) * 512, 512), 512)], preferred_element_type=jnp.float32)
                q = (q * QSCALE).astype(jnp.bfloat16)
                for j in range(4):
                    q_s[s, (t & 1) * 4 + j] = q[:, j * Dh:(j + 1) * Dh]
                return 0
            jax.lax.fori_loop(0, 2 * QA, q0, 0)

        with ns("P_mainloop"):
            UQ = (NS - QA) * OB
            UV = NUNITS - LD
            UK = NUNITS - LP
            jax.lax.fori_loop(0, OB, make_step(True, False, events=False, do_w=True), 0)
            jax.lax.fori_loop(OB, UQ, make_step(True, True, do_w=True), 0)
            jax.lax.fori_loop(UQ, UV, make_step(False, True), 0)
            jax.lax.fori_loop(UV, UK, make_step(False, True, do_v=False, events=False, tail=True), 0)
            for u in range(UK, NUNITS - 1):
                make_step(False, True, do_k=False, do_v=False, events=False)(u, 0)

        u = NUNITS - 1
        with ns("P_wait_k127"):
            for g in range(G):
                k_cp(u, g).wait()
        with ns("P_q127"):
            opiece(NS - 2, OB - 1)
            pls = [sm(sc) for sc in qk(u)]
        with ns("P_wait_v127"):
            v_cp(u).wait()
            out_cp(0, EARLY, 0).start()
        with ns("P_p127"):
            for t in range(2):
                pvf(u, t, *pls[t])
        with ns("P_oproj_last"):
            oproj_tail(EARLY, LASTN)
            out_cp(EARLY, LASTN, 1).start()
        with ns("P_final"):
            out_cp(0, EARLY, 0).wait()
            out_cp(EARLY, LASTN, 1).wait()

    @jax.jit
    def f(x, k_cache, v_cache, wq, wo):
        x2 = x.reshape(ROWS, D)
        out = pl.pallas_call(
            kernel,
            out_shape=jax.ShapeDtypeStruct((ROWS, D), jnp.bfloat16),
            in_specs=[pl.BlockSpec(memory_space=pl.ANY)] * 5,
            out_specs=pl.BlockSpec(memory_space=pl.ANY),
            scratch_shapes=[
                pltpu.VMEM((ROWS, D), jnp.bfloat16),
                pltpu.VMEM((Hkv + 1, D, GW), jnp.bfloat16),
                pltpu.VMEM((Hkv + 1, GW, D), jnp.bfloat16),
                pltpu.VMEM((NK, Sk, Dh), jnp.bfloat16),
                pltpu.VMEM((NV, Sk, Dh), jnp.bfloat16),
                pltpu.VMEM((NQ, REP, CH, Dh), jnp.bfloat16),
                pltpu.VMEM((2, REP, CH, Dh), jnp.bfloat16),
                pltpu.VMEM((ROWS, D), jnp.float32),
                pltpu.VMEM((ROWS, D), jnp.bfloat16),
                pltpu.SemaphoreType.DMA((1,)),
                pltpu.SemaphoreType.DMA((Hkv,)),
                pltpu.SemaphoreType.DMA((Hkv,)),
                pltpu.SemaphoreType.DMA((NK, G)),
                pltpu.SemaphoreType.DMA((NV,)),
                pltpu.SemaphoreType.DMA((2,)),
            ],
            compiler_params=pltpu.CompilerParams(vmem_limit_bytes=100 * 1024 * 1024, disable_bounds_checks=nobounds),
        )(x2, k_cache, v_cache, wq, wo)
        return out.reshape(B, Sq, D)
    return f

pallas_standalone__gqa_block_cached__sampling_kernel = make(wprio=1)
```

```python
import math

import jax
import jax.numpy as jnp
import jax.experimental.pallas as pl
import jax.experimental.pallas.tpu as pltpu

_B, _SQ, _D = 32, 16, 1024
_HQ, _HKV, _SK, _DH = 32, 4, 2048, 128
_REP = _HQ // _HKV
_GW = _REP * _DH
_ROWS = _B * _SQ
_NUNITS = _B * _HKV
_STEP_UNITS = 8
_STEP_ROWS = _STEP_UNITS * _SQ
_HALF_ROWS = _STEP_ROWS // 2
_NSTEPS = _NUNITS // _STEP_UNITS
_QA = 3
_QSCALE = (_DH ** -0.5) * math.log2(math.e)
_NT = (((1,), (1,)), ((), ()))

_NQ, _NK, _NV = 4, 16, 16
_LK = 2
_LV = 10
_KP = 8
_KP_ROWS = _SK // _KP
_WP_ROWS = 64
_U_INORDER = 122
_U_SPLIT = 124
_EARLY_ROWS = _ROWS - _HALF_ROWS

_AT_FIRST = ("top", "sA7", "sA15", "sB7", "sB15", "oA", "oB", "q")
_AT_MAIN = ("top", "sA15", "sB7", "sB15", "oA", "oB", "y", "q")
_AT_NOQ = ("top", "sA7", "sA15", "sB7", "sB15", "oA", "oB", "y")
_AT_SPLIT = ("top", "y", "sA15", "sB7", "sB15", "mid", "oA", "oB")
_AT_WO, _AT_WQ = "sA7", "pB7"
_FIRST_REQUESTS = "VVVoVVqVVVVV"


def _kernel(x_hbm, k_hbm, v_hbm, wq_hbm, wo_hbm, out_hbm,
            x_buf, wq_buf, wo_buf, k_buf, v_buf, q_s, o_s, acc, out_buf,
            x_sem, wq_sem, wo_sem, k_sem, v_sem, out_sem):
    def x_cp():
        return pltpu.make_async_copy(x_hbm, x_buf, x_sem.at[0])

    def wq_cp(h):
        cols = pl.ds(pl.multiple_of(h * _GW, _GW), _GW)
        return pltpu.make_async_copy(wq_hbm.at[:, cols], wq_buf.at[h], wq_sem.at[h])

    def wo_cp(h):
        rows = pl.ds(pl.multiple_of(h * _GW, _GW), _GW)
        return pltpu.make_async_copy(wo_hbm.at[rows, :], wo_buf.at[h], wo_sem.at[h])

    def wq_piece(h, j):
        rows = pl.ds(pl.multiple_of(j * _WP_ROWS, _WP_ROWS), _WP_ROWS)
        cols = pl.ds(pl.multiple_of(h * _GW, _GW), _GW)
        return pltpu.make_async_copy(wq_hbm.at[rows, cols], wq_buf.at[h, rows], wq_sem.at[h])

    def wo_piece(h, j):
        src = pl.ds(pl.multiple_of(h * _GW + j * _WP_ROWS, _WP_ROWS), _WP_ROWS)
        dst = pl.ds(pl.multiple_of(j * _WP_ROWS, _WP_ROWS), _WP_ROWS)
        return pltpu.make_async_copy(wo_hbm.at[src, :], wo_buf.at[h, dst], wo_sem.at[h])

    def k_cp(u):
        slot = u & (_NK - 1)
        return pltpu.make_async_copy(k_hbm.at[u & (_B - 1), u >> 5], k_buf.at[slot], k_sem.at[slot])

    def k_piece(u, g):
        slot = u & (_NK - 1)
        rows = pl.ds(g * _KP_ROWS, _KP_ROWS)
        return pltpu.make_async_copy(
            k_hbm.at[u & (_B - 1), u >> 5, rows], k_buf.at[slot, rows], k_sem.at[slot])

    def v_cp(u):
        slot = u & (_NV - 1)
        return pltpu.make_async_copy(v_hbm.at[u & (_B - 1), u >> 5], v_buf.at[slot], v_sem.at[slot])

    def out_cp(r0, n, i):
        rows = pl.ds(r0, n)
        return pltpu.make_async_copy(out_buf.at[rows, :], out_hbm.at[rows, :], out_sem.at[i])

    def step_rows(s):
        return pl.ds(pl.multiple_of((s & 3) * _STEP_ROWS, _STEP_ROWS), _STEP_ROWS)

    def q_piece(s, i):
        cols = pl.ds(pl.multiple_of(i * _DH, _DH), _DH)
        q = jnp.dot(x_buf[step_rows(s), :], wq_buf[s >> 2, :, cols], preferred_element_type=jnp.float32)
        q = (q * _QSCALE).astype(jnp.bfloat16)
        q_s[s & (_NQ - 1), i] = q
        return q

    def o_piece(t, i):
        rows = pl.ds(pl.multiple_of((t & 7) * _HALF_ROWS, _HALF_ROWS), _HALF_ROWS)
        cols = pl.ds(pl.multiple_of(i * (_D // 4), _D // 4), _D // 4)
        o = jnp.concatenate([o_s[t & 1, j] for j in range(_REP)], axis=1)
        y = jnp.dot(o, wo_buf[t >> 3, :, cols], preferred_element_type=jnp.float32)
        a = acc[rows, cols] + y
        acc[rows, cols] = a
        out_buf[rows, cols] = a.astype(jnp.bfloat16)
        return y

    def scores(u):
        s = u >> 3
        rows = pl.ds(pl.multiple_of((u & (_STEP_UNITS - 1)) * _SQ, _SQ), _SQ)
        k = k_buf[u & (_NK - 1)]
        out = []
        for t in range(2):
            heads = range(t * _REP // 2, (t + 1) * _REP // 2)
            q = jnp.concatenate([q_s[s & (_NQ - 1), j, rows, :] for j in heads], axis=0)
            out.append(jax.lax.dot_general(q, k, _NT, preferred_element_type=jnp.float32))
        return out

    def softmax(sc):
        m = jnp.max(sc, axis=1, keepdims=True)
        p = jnp.exp2(sc - m)
        return p.astype(jnp.bfloat16), jnp.sum(p, axis=1, keepdims=True)

    def attend(u, t, p, l):
        rows = pl.ds(pl.multiple_of((u & 3) * _SQ, _SQ), _SQ)
        o = jnp.dot(p, v_buf[u & (_NV - 1)], preferred_element_type=jnp.float32)
        o = (o * (1.0 / l)).astype(jnp.bfloat16)
        for j in range(_REP // 2):
            o_s[(u >> 2) & 1, t * (_REP // 2) + j, rows, :] = o[j * _SQ:(j + 1) * _SQ, :]
        return o

    def await_weights(u):
        g = u >> 5

        @pl.when((u & (_B - 1)) == 4)
        def _():
            wo_cp(g).wait()

        @pl.when(jnp.logical_and((u & (_B - 1)) == _STEP_UNITS, g < _HKV - 1))
        def _():
            wq_cp(g + 1).wait()

    def make_unit(at, *, do_q, do_o, do_w=False, last_phase=False, split=False):
        def unit(u, carry):
            n = u + _LK
            seen = []

            def request(name, val=None):
                if name in at:
                    g = at.index(name)
                    seen.append(name)
                    if val is not None:
                        k_buf[_NK, pl.ds(0, _SQ), :] = val[:_SQ, :_DH].astype(jnp.bfloat16)
                    if last_phase:
                        pl.when(n < _U_INORDER)(lambda: k_piece(n, g).start(priority=0))
                    else:
                        k_piece(n, g).start(priority=0)
                if do_w and name in (_AT_WO, _AT_WQ):
                    h = u >> 5
                    j = u & (_B - 1)
                    if name == _AT_WO:
                        wo_buf[_HKV, pl.ds(0, _SQ), pl.ds(0, _DH)] = val[:_SQ, :_DH].astype(jnp.bfloat16)
                        pl.when(jnp.logical_and(h < _HKV - 1, j < _GW // _WP_ROWS))(
                            lambda: wo_piece(h + 1, j).start(priority=1))
                    else:
                        wq_buf[_HKV, pl.ds(0, _SQ), pl.ds(0, _DH)] = val[:_SQ, :_DH].astype(jnp.bfloat16)
                        pl.when(jnp.logical_and(h < _HKV - 2, j < _D // _WP_ROWS))(
                            lambda: wq_piece(h + 2, j).start(priority=1))

            if do_o:
                pl.when((u & 3) == 0)(lambda: await_weights(u))
            k_cp(u).wait()
            if not split:
                v_cp(u).wait()
            if last_phase:
                pl.when(jnp.logical_and(u + _LV >= _U_INORDER, u + _LV < _NUNITS))(
                    lambda: k_cp(u + _LV).start(priority=1))
            request("top")
            if split:
                request("y", o_piece((u >> 2) - 1, u & 3))
            sa, sb = scores(u)
            request("sA7", sa[:, 7 * _DH:])
            request("sA15", sa[:, 15 * _DH:])
            request("sB7", sb[:, 7 * _DH:])
            request("sB15", sb[:, 15 * _DH:])
            pa, la = softmax(sa)
            if split:
                v_cp(u).wait()
                pl.when(u == _NUNITS - 1)(lambda: out_cp(0, _EARLY_ROWS, 0).start())
            request("mid")
            pb, lb = softmax(sb)
            request("pB7", pb[:, 7 * _DH:])
            request("oA", attend(u, 0, pa, la))
            request("oB", attend(u, 1, pb, lb))
            if do_o and not split:
                request("y", o_piece((u >> 2) - 1, u & 3))
            if do_q:
                request("q", q_piece((u >> 3) + _QA, u & (_STEP_UNITS - 1)))
            if last_phase:
                pl.when(u + _LV < _NUNITS)(lambda: v_cp(u + _LV).start(priority=1))
            else:
                v_cp(u + _LV).start(priority=1)
            assert sorted(seen) == sorted(at), (seen, at)
            return carry

        return unit

    x_cp().start()
    wq_cp(0).start()

    def first_k(n, carry):
        for g in range(_KP):
            k_piece(n, g).start(priority=0)
        return carry

    jax.lax.fori_loop(0, _LK, first_k, 0)

    def first_low(j, carry):
        n_v = 0
        for jj, what in enumerate(_FIRST_REQUESTS):
            if what == "V":
                pl.when(j == jj)(lambda n_v=n_v: v_cp(n_v).start(priority=1))
                n_v += 1
            elif what == "q":
                pl.when(j == jj)(lambda: wq_cp(1).start(priority=1))
            else:
                pl.when(j == jj)(lambda: wo_cp(0).start(priority=1))
        return carry

    jax.lax.fori_loop(0, len(_FIRST_REQUESTS), first_low, 0)
    acc[...] = jnp.zeros_like(acc)
    x_cp().wait()
    wq_cp(0).wait()

    def first_q(t, carry):
        s = t >> 1
        cols = pl.ds(pl.multiple_of((t & 1) * (_GW // 2), _GW // 2), _GW // 2)
        q = jnp.dot(x_buf[step_rows(s), :], wq_buf[0, :, cols], preferred_element_type=jnp.float32)
        q = (q * _QSCALE).astype(jnp.bfloat16)
        for j in range(_REP // 2):
            q_s[s, (t & 1) * (_REP // 2) + j] = q[:, j * _DH:(j + 1) * _DH]
        return carry

    jax.lax.fori_loop(0, 2 * _QA, first_q, 0)

    u_noq = (_NSTEPS - _QA) * _STEP_UNITS
    assert _FIRST_REQUESTS.count("V") == _LV and u_noq + _LV <= _U_INORDER <= _U_SPLIT + _LK
    jax.lax.fori_loop(0, 4, make_unit(_AT_FIRST, do_q=True, do_o=False, do_w=True), 0)
    jax.lax.fori_loop(4, u_noq, make_unit(_AT_MAIN, do_q=True, do_o=True, do_w=True), 0)
    jax.lax.fori_loop(u_noq, _U_SPLIT, make_unit(_AT_NOQ, do_q=False, do_o=True, last_phase=True), 0)
    jax.lax.fori_loop(
        _U_SPLIT, _NUNITS, make_unit(_AT_SPLIT, do_q=False, do_o=True, last_phase=True, split=True), 0)

    o = jnp.concatenate([o_s[1, j] for j in range(_REP)], axis=1)
    y = jnp.dot(o, wo_buf[_HKV - 1], preferred_element_type=jnp.float32)
    last = pl.ds(_EARLY_ROWS, _HALF_ROWS)
    out_buf[last, :] = (acc[last, :] + y).astype(jnp.bfloat16)
    out_cp(_EARLY_ROWS, _HALF_ROWS, 1).start()
    out_cp(0, _EARLY_ROWS, 0).wait()
    out_cp(_EARLY_ROWS, _HALF_ROWS, 1).wait()


@jax.jit
def pallas_standalone__gqa_block_cached__sampling_kernel(
    x: jax.Array,
    k_cache: jax.Array,
    v_cache: jax.Array,
    wq: jax.Array,
    wo: jax.Array,
):
    assert x.shape == (_B, _SQ, _D) and k_cache.shape == v_cache.shape == (_B, _HKV, _SK, _DH)
    assert wq.shape == (_D, _HQ * _DH) and wo.shape == (_HQ * _DH, _D)
    bf16 = jnp.bfloat16
    out = pl.pallas_call(
        _kernel,
        out_shape=jax.ShapeDtypeStruct((_ROWS, _D), bf16),
        in_specs=[pl.BlockSpec(memory_space=pl.ANY)] * 5,
        out_specs=pl.BlockSpec(memory_space=pl.ANY),
        scratch_shapes=[
            pltpu.VMEM((_ROWS, _D), bf16),
            pltpu.VMEM((_HKV + 1, _D, _GW), bf16),
            pltpu.VMEM((_HKV + 1, _GW, _D), bf16),
            pltpu.VMEM((_NK + 1, _SK, _DH), bf16),
            pltpu.VMEM((_NV, _SK, _DH), bf16),
            pltpu.VMEM((_NQ, _REP, _STEP_ROWS, _DH), bf16),
            pltpu.VMEM((2, _REP, _HALF_ROWS, _DH), bf16),
            pltpu.VMEM((_ROWS, _D), jnp.float32),
            pltpu.VMEM((_ROWS, _D), bf16),
            pltpu.SemaphoreType.DMA((1,)),
            pltpu.SemaphoreType.DMA((_HKV,)),
            pltpu.SemaphoreType.DMA((_HKV,)),
            pltpu.SemaphoreType.DMA((_NK,)),
            pltpu.SemaphoreType.DMA((_NV,)),
            pltpu.SemaphoreType.DMA((2,)),
        ],
        compiler_params=pltpu.CompilerParams(
            vmem_limit_bytes=100 * 1024 * 1024,
            disable_bounds_checks=True,
            disable_semaphore_checks=True,
        ),
    )(x.reshape(_ROWS, _D).astype(bf16), k_cache.astype(bf16), v_cache.astype(bf16),
      wq.astype(bf16), wo.astype(bf16))
    return out.reshape(_B, _SQ, _D).astype(x.dtype)
```

```python
import math

import jax
import jax.numpy as jnp
import jax.experimental.pallas as pl
import jax.experimental.pallas.tpu as pltpu

_B, _SQ, _D = 32, 16, 1024
_HQ, _HKV, _SK, _DH = 32, 4, 2048, 128
_REP = _HQ // _HKV
_GW = _REP * _DH
_ROWS = _B * _SQ
_NUNITS = _B * _HKV
_STEP_UNITS = 8
_STEP_ROWS = _STEP_UNITS * _SQ
_HALF_ROWS = _STEP_ROWS // 2
_NSTEPS = _NUNITS // _STEP_UNITS
_QA = 3
_QSCALE = (_DH ** -0.5) * math.log2(math.e)
_NT = (((1,), (1,)), ((), ()))

_NQ, _NK, _NV = 4, 16, 16
_LK = 2
_LV = 8
_KP = 8
_KP_ROWS = _SK // _KP
_WP_ROWS = 64
_U_INORDER = 122
_U_SPLIT = 124
_EARLY_ROWS = _ROWS - _HALF_ROWS

_AT_FIRST = ("top", "sA7", "sA15", "sB7", "sB15", "oA", "oB", "q")
_AT_MAIN = ("top", "sA15", "sB7", "sB15", "oA", "oB", "y", "q")
_AT_NOQ = ("top", "sA7", "sA15", "sB7", "sB15", "oA", "oB", "y")
_AT_SPLIT = ("top", "y", "sA15", "sB7", "sB15", "mid", "oA", "oB")
_AT_WO, _AT_WQ = "sA7", "pB7"
_FIRST_REQUESTS = "VVVoVVqVVV"
_NP0 = 32


def _kernel(x_hbm, k_hbm, v_hbm, wq_hbm, wo_hbm, out_hbm,
            x_buf, wq_buf, wo_buf, k_buf, v_buf, q_s, o_s, acc, out_buf,
            x_sem, wq_sem, wo_sem, k_sem, v_sem, out_sem, wq0_sem):
    def x_cp():
        return pltpu.make_async_copy(x_hbm, x_buf, x_sem.at[0])

    def wq_cp(h):
        cols = pl.ds(pl.multiple_of(h * _GW, _GW), _GW)
        return pltpu.make_async_copy(wq_hbm.at[:, cols], wq_buf.at[h], wq_sem.at[h])

    def wo_cp(h):
        rows = pl.ds(pl.multiple_of(h * _GW, _GW), _GW)
        return pltpu.make_async_copy(wo_hbm.at[rows, :], wo_buf.at[h], wo_sem.at[h])

    def wq_piece(h, j):
        rows = pl.ds(pl.multiple_of(j * _WP_ROWS, _WP_ROWS), _WP_ROWS)
        cols = pl.ds(pl.multiple_of(h * _GW, _GW), _GW)
        return pltpu.make_async_copy(wq_hbm.at[rows, cols], wq_buf.at[h, rows], wq_sem.at[h])

    def wo_piece(h, j):
        src = pl.ds(pl.multiple_of(h * _GW + j * _WP_ROWS, _WP_ROWS), _WP_ROWS)
        dst = pl.ds(pl.multiple_of(j * _WP_ROWS, _WP_ROWS), _WP_ROWS)
        return pltpu.make_async_copy(wo_hbm.at[src, :], wo_buf.at[h, dst], wo_sem.at[h])

    def k_cp(u):
        slot = u & (_NK - 1)
        return pltpu.make_async_copy(k_hbm.at[u & (_B - 1), u >> 5], k_buf.at[slot], k_sem.at[slot])

    def k_piece(u, g):
        slot = u & (_NK - 1)
        rows = pl.ds(g * _KP_ROWS, _KP_ROWS)
        return pltpu.make_async_copy(
            k_hbm.at[u & (_B - 1), u >> 5, rows], k_buf.at[slot, rows], k_sem.at[slot])

    def v_cp(u):
        slot = u & (_NV - 1)
        return pltpu.make_async_copy(v_hbm.at[u & (_B - 1), u >> 5], v_buf.at[slot], v_sem.at[slot])

    def out_cp(r0, n, i):
        rows = pl.ds(r0, n)
        return pltpu.make_async_copy(out_buf.at[rows, :], out_hbm.at[rows, :], out_sem.at[i])

    def step_rows(s):
        return pl.ds(pl.multiple_of((s & 3) * _STEP_ROWS, _STEP_ROWS), _STEP_ROWS)

    def q_piece(s, i):
        cols = pl.ds(pl.multiple_of(i * _DH, _DH), _DH)
        q = jnp.dot(x_buf[step_rows(s), :], wq_buf[s >> 2, :, cols], preferred_element_type=jnp.float32)
        q = (q * _QSCALE).astype(jnp.bfloat16)
        q_s[s & (_NQ - 1), i] = q
        return q

    def o_piece(t, i):
        rows = pl.ds(pl.multiple_of((t & 7) * _HALF_ROWS, _HALF_ROWS), _HALF_ROWS)
        cols = pl.ds(pl.multiple_of(i * (_D // 4), _D // 4), _D // 4)
        o = jnp.concatenate([o_s[t & 1, j] for j in range(_REP)], axis=1)
        y = jnp.dot(o, wo_buf[t >> 3, :, cols], preferred_element_type=jnp.float32)
        a = acc[rows, cols] + y
        acc[rows, cols] = a
        out_buf[rows, cols] = a.astype(jnp.bfloat16)
        return y

    def scores(u):
        s = u >> 3
        rows = pl.ds(pl.multiple_of((u & (_STEP_UNITS - 1)) * _SQ, _SQ), _SQ)
        k = k_buf[u & (_NK - 1)]
        out = []
        for t in range(2):
            heads = range(t * _REP // 2, (t + 1) * _REP // 2)
            q = jnp.concatenate([q_s[s & (_NQ - 1), j, rows, :] for j in heads], axis=0)
            out.append(jax.lax.dot_general(q, k, _NT, preferred_element_type=jnp.float32))
        return out

    def softmax(sc):
        m = jnp.max(sc, axis=1, keepdims=True)
        p = jnp.exp2(sc - m)
        return p.astype(jnp.bfloat16), jnp.sum(p, axis=1, keepdims=True)

    def attend(u, t, p, l):
        rows = pl.ds(pl.multiple_of((u & 3) * _SQ, _SQ), _SQ)
        o = jnp.dot(p, v_buf[u & (_NV - 1)], preferred_element_type=jnp.float32)
        o = (o * (1.0 / l)).astype(jnp.bfloat16)
        for j in range(_REP // 2):
            o_s[(u >> 2) & 1, t * (_REP // 2) + j, rows, :] = o[j * _SQ:(j + 1) * _SQ, :]
        return o

    def await_weights(u):
        g = u >> 5

        @pl.when((u & (_B - 1)) == 4)
        def _():
            wo_cp(g).wait()

        @pl.when(jnp.logical_and((u & (_B - 1)) == _STEP_UNITS, g < _HKV - 1))
        def _():
            wq_cp(g + 1).wait()

    def make_unit(at, *, do_q, do_o, do_w=False, last_phase=False, split=False):
        def unit(u, carry):
            n = u + _LK
            seen = []

            def request(name, val=None):
                if name in at:
                    g = at.index(name)
                    seen.append(name)
                    if val is not None:
                        k_buf[_NK, pl.ds(0, _SQ), :] = val[:_SQ, :_DH].astype(jnp.bfloat16)
                    if last_phase:
                        pl.when(n < _U_INORDER)(lambda: k_piece(n, g).start(priority=0))
                    else:
                        k_piece(n, g).start(priority=0)
                if do_w and name in (_AT_WO, _AT_WQ):
                    h = u >> 5
                    j = u & (_B - 1)
                    if name == _AT_WO:
                        wo_buf[_HKV, pl.ds(0, _SQ), pl.ds(0, _DH)] = val[:_SQ, :_DH].astype(jnp.bfloat16)
                        pl.when(jnp.logical_and(h < _HKV - 1, j < _GW // _WP_ROWS))(
                            lambda: wo_piece(h + 1, j).start(priority=1))
                    else:
                        wq_buf[_HKV, pl.ds(0, _SQ), pl.ds(0, _DH)] = val[:_SQ, :_DH].astype(jnp.bfloat16)
                        pl.when(jnp.logical_and(h < _HKV - 2, j < _D // _WP_ROWS))(
                            lambda: wq_piece(h + 2, j).start(priority=1))

            if do_o:
                pl.when((u & 3) == 0)(lambda: await_weights(u))
            k_cp(u).wait()
            if not split:
                v_cp(u).wait()
            if last_phase:
                pl.when(jnp.logical_and(u + _LV >= _U_INORDER, u + _LV < _NUNITS))(
                    lambda: k_cp(u + _LV).start(priority=1))
            request("top")
            if split:
                request("y", o_piece((u >> 2) - 1, u & 3))
            sa, sb = scores(u)
            request("sA7", sa[:, 7 * _DH:])
            request("sA15", sa[:, 15 * _DH:])
            request("sB7", sb[:, 7 * _DH:])
            request("sB15", sb[:, 15 * _DH:])
            pa, la = softmax(sa)
            if split:
                v_cp(u).wait()
                pl.when(u == _NUNITS - 1)(lambda: out_cp(0, _EARLY_ROWS, 0).start())
            request("mid")
            pb, lb = softmax(sb)
            request("pB7", pb[:, 7 * _DH:])
            request("oA", attend(u, 0, pa, la))
            request("oB", attend(u, 1, pb, lb))
            if do_o and not split:
                request("y", o_piece((u >> 2) - 1, u & 3))
            if do_q:
                request("q", q_piece((u >> 3) + _QA, u & (_STEP_UNITS - 1)))
            if last_phase:
                pl.when(u + _LV < _NUNITS)(lambda: v_cp(u + _LV).start(priority=1))
            else:
                v_cp(u + _LV).start(priority=1)
            assert sorted(seen) == sorted(at), (seen, at)
            return carry

        return unit

    def x_piece(j):
        rows = pl.ds(pl.multiple_of(j * (_ROWS // _NP0), _ROWS // _NP0), _ROWS // _NP0)
        return pltpu.make_async_copy(x_hbm.at[rows, :], x_buf.at[rows, :], x_sem.at[0])

    def wq0_piece(j):
        rows = pl.ds(pl.multiple_of(j * (_D // _NP0), _D // _NP0), _D // _NP0)
        return pltpu.make_async_copy(wq_hbm.at[rows, pl.ds(0, _GW)], wq_buf.at[0, rows], wq0_sem.at[j])

    def first_k_piece(p):
        n = p >> 3
        rows = pl.ds(pl.multiple_of((p & (_KP - 1)) * _KP_ROWS, _KP_ROWS), _KP_ROWS)
        return pltpu.make_async_copy(k_hbm.at[n, 0, rows], k_buf.at[n, rows], k_sem.at[n])

    x_piece(0).start(priority=0)

    def first_wq(j, carry):
        wq0_piece(j).start(priority=1)
        return carry

    jax.lax.fori_loop(0, _NP0, first_wq, 0)

    def first_low(j, carry):
        n_v = 0
        for jj, what in enumerate(_FIRST_REQUESTS):
            if what == "V":
                pl.when(j == jj)(lambda n_v=n_v: v_cp(n_v).start(priority=1))
                n_v += 1
            elif what == "q":
                pl.when(j == jj)(lambda: wq_cp(1).start(priority=1))
            else:
                pl.when(j == jj)(lambda: wo_cp(0).start(priority=1))
        return carry

    jax.lax.fori_loop(0, len(_FIRST_REQUESTS), first_low, 0)
    acc[...] = jnp.zeros_like(acc)

    def first_x(j, carry):
        wq0_piece(j).wait()
        pl.when(j + 1 < _NP0)(lambda: x_piece(j + 1).start(priority=0))
        return carry

    jax.lax.fori_loop(0, _NP0, first_x, 0)
    x_cp().wait()

    def first_q(t, carry):
        s = t >> 1
        cols = pl.ds(pl.multiple_of((t & 1) * (_GW // 2), _GW // 2), _GW // 2)
        first_k_piece(3 * t).start(priority=0)
        q = jnp.dot(x_buf[step_rows(s), :], wq_buf[0, :, cols], preferred_element_type=jnp.float32)
        q = (q * _QSCALE).astype(jnp.bfloat16)
        for i, j in ((1, 1), (2, 3)):
            k_buf[_NK, pl.ds(0, _SQ), :] = q[:_SQ, j * _DH:(j + 1) * _DH]
            pl.when(3 * t + i < _LK * _KP)(lambda i=i: first_k_piece(3 * t + i).start(priority=0))
        for j in range(_REP // 2):
            q_s[s, (t & 1) * (_REP // 2) + j] = q[:, j * _DH:(j + 1) * _DH]
        return carry

    assert 3 * (2 * _QA - 1) < _LK * _KP <= 3 * 2 * _QA
    jax.lax.fori_loop(0, 2 * _QA, first_q, 0)

    u_noq = (_NSTEPS - _QA) * _STEP_UNITS
    assert _FIRST_REQUESTS.count("V") == _LV and u_noq + _LV <= _U_INORDER <= _U_SPLIT + _LK
    jax.lax.fori_loop(0, 4, make_unit(_AT_FIRST, do_q=True, do_o=False, do_w=True), 0)
    jax.lax.fori_loop(4, u_noq, make_unit(_AT_MAIN, do_q=True, do_o=True, do_w=True), 0)
    jax.lax.fori_loop(u_noq, _U_SPLIT, make_unit(_AT_NOQ, do_q=False, do_o=True, last_phase=True), 0)
    jax.lax.fori_loop(
        _U_SPLIT, _NUNITS, make_unit(_AT_SPLIT, do_q=False, do_o=True, last_phase=True, split=True), 0)

    o = jnp.concatenate([o_s[1, j] for j in range(_REP)], axis=1)
    y = jnp.dot(o, wo_buf[_HKV - 1], preferred_element_type=jnp.float32)
    last = pl.ds(_EARLY_ROWS, _HALF_ROWS)
    out_buf[last, :] = (acc[last, :] + y).astype(jnp.bfloat16)
    out_cp(_EARLY_ROWS, _HALF_ROWS, 1).start()
    out_cp(0, _EARLY_ROWS, 0).wait()
    out_cp(_EARLY_ROWS, _HALF_ROWS, 1).wait()


@jax.jit
def pallas_standalone__gqa_block_cached__sampling_kernel(
    x: jax.Array,
    k_cache: jax.Array,
    v_cache: jax.Array,
    wq: jax.Array,
    wo: jax.Array,
):
    assert x.shape == (_B, _SQ, _D) and k_cache.shape == v_cache.shape == (_B, _HKV, _SK, _DH)
    assert wq.shape == (_D, _HQ * _DH) and wo.shape == (_HQ * _DH, _D)
    bf16 = jnp.bfloat16
    out = pl.pallas_call(
        _kernel,
        out_shape=jax.ShapeDtypeStruct((_ROWS, _D), bf16),
        in_specs=[pl.BlockSpec(memory_space=pl.ANY)] * 5,
        out_specs=pl.BlockSpec(memory_space=pl.ANY),
        scratch_shapes=[
            pltpu.VMEM((_ROWS, _D), bf16),
            pltpu.VMEM((_HKV + 1, _D, _GW), bf16),
            pltpu.VMEM((_HKV + 1, _GW, _D), bf16),
            pltpu.VMEM((_NK + 1, _SK, _DH), bf16),
            pltpu.VMEM((_NV, _SK, _DH), bf16),
            pltpu.VMEM((_NQ, _REP, _STEP_ROWS, _DH), bf16),
            pltpu.VMEM((2, _REP, _HALF_ROWS, _DH), bf16),
            pltpu.VMEM((_ROWS, _D), jnp.float32),
            pltpu.VMEM((_ROWS, _D), bf16),
            pltpu.SemaphoreType.DMA((1,)),
            pltpu.SemaphoreType.DMA((_HKV,)),
            pltpu.SemaphoreType.DMA((_HKV,)),
            pltpu.SemaphoreType.DMA((_NK,)),
            pltpu.SemaphoreType.DMA((_NV,)),
            pltpu.SemaphoreType.DMA((2,)),
            pltpu.SemaphoreType.DMA((_NP0,)),
        ],
        compiler_params=pltpu.CompilerParams(
            vmem_limit_bytes=100 * 1024 * 1024,
            disable_semaphore_checks=True,
        ),
    )(x.reshape(_ROWS, _D).astype(bf16), k_cache.astype(bf16), v_cache.astype(bf16),
      wq.astype(bf16), wo.astype(bf16))
    return out.reshape(_B, _SQ, _D).astype(x.dtype)
```

```python
import math

import jax
import jax.numpy as jnp
import jax.experimental.pallas as pl
import jax.experimental.pallas.tpu as pltpu

_B, _SQ, _D = 32, 16, 1024
_HQ, _HKV, _SK, _DH = 32, 4, 2048, 128
_REP = _HQ // _HKV
_GW = _REP * _DH
_ROWS = _B * _SQ
_NUNITS = _B * _HKV
_STEP_UNITS = 8
_STEP_ROWS = _STEP_UNITS * _SQ
_HALF_ROWS = _STEP_ROWS // 2
_NSTEPS = _NUNITS // _STEP_UNITS
_QA = 3
_QSCALE = (_DH ** -0.5) * math.log2(math.e)
_NT = (((1,), (1,)), ((), ()))

_NQ, _NK, _NV = 4, 16, 16
_LK = 2
_LV = 5
_VP_ROWS = (768, 768, 512)
_KP0, _KP0_ROWS = 8, _SK // 8
_WP_ROWS = 64
_U_INORDER = 122
_U_SPLIT = 124
_EARLY_ROWS = _ROWS - _HALF_ROWS

_AT_FIRST = (("v0", 256), ("v1", 256), ("top", 128), ("sA15", 256), ("sB7", 256), ("sB15", 256),
             ("oA", 256), ("oB", 256), ("q", 128))
_AT_MAIN = (("v0", 256), ("v1", 256), ("top", 128), ("sA15", 128), ("sB7", 128), ("sB15", 256),
            ("oA", 256), ("oB", 256), ("y", 256), ("q", 128))
_AT_NOQ = (("v0", 256), ("v1", 256), ("top", 128), ("sA15", 256), ("sB7", 256), ("sB15", 256),
           ("oA", 256), ("oB", 256), ("y", 128))
_AT_SPLIT = (("top", 256), ("y", 256), ("sA15", 256), ("sB7", 256), ("sB15", 256), ("mid", 256),
             ("oA", 256), ("oB", 256))
_AT_WO, _AT_WQ = "sA7", "pB7"
_FIRST_REQUESTS = "VVVoVqV"
_NP0 = 32


def _kernel(x_hbm, k_hbm, v_hbm, wq_hbm, wo_hbm, out_hbm,
            x_buf, wq_buf, wo_buf, k_buf, v_buf, q_s, o_s, acc, out_buf,
            x_sem, wq_sem, wo_sem, k_sem, v_sem, out_sem, wq0_sem):
    def x_cp():
        return pltpu.make_async_copy(x_hbm, x_buf, x_sem.at[0])

    def wq_cp(h):
        cols = pl.ds(pl.multiple_of(h * _GW, _GW), _GW)
        return pltpu.make_async_copy(wq_hbm.at[:, cols], wq_buf.at[h], wq_sem.at[h])

    def wo_cp(h):
        rows = pl.ds(pl.multiple_of(h * _GW, _GW), _GW)
        return pltpu.make_async_copy(wo_hbm.at[rows, :], wo_buf.at[h], wo_sem.at[h])

    def wq_piece(h, j):
        rows = pl.ds(pl.multiple_of(j * _WP_ROWS, _WP_ROWS), _WP_ROWS)
        cols = pl.ds(pl.multiple_of(h * _GW, _GW), _GW)
        return pltpu.make_async_copy(wq_hbm.at[rows, cols], wq_buf.at[h, rows], wq_sem.at[h])

    def wo_piece(h, j):
        src = pl.ds(pl.multiple_of(h * _GW + j * _WP_ROWS, _WP_ROWS), _WP_ROWS)
        dst = pl.ds(pl.multiple_of(j * _WP_ROWS, _WP_ROWS), _WP_ROWS)
        return pltpu.make_async_copy(wo_hbm.at[src, :], wo_buf.at[h, dst], wo_sem.at[h])

    def k_cp(u):
        slot = u & (_NK - 1)
        return pltpu.make_async_copy(k_hbm.at[u & (_B - 1), u >> 5], k_buf.at[slot], k_sem.at[slot])

    def k_piece(u, r0, n):
        slot = u & (_NK - 1)
        rows = pl.ds(r0, n)
        return pltpu.make_async_copy(
            k_hbm.at[u & (_B - 1), u >> 5, rows], k_buf.at[slot, rows], k_sem.at[slot])

    def v_part(u, j):
        slot = u & (_NV - 1)
        rows = pl.ds(sum(_VP_ROWS[:j]), _VP_ROWS[j])
        return pltpu.make_async_copy(
            v_hbm.at[u & (_B - 1), u >> 5, rows], v_buf.at[slot, rows], v_sem.at[slot, j])

    def v_start(u):
        for j in range(len(_VP_ROWS)):
            v_part(u, j).start(priority=1)

    def out_cp(r0, n, i):
        rows = pl.ds(r0, n)
        return pltpu.make_async_copy(out_buf.at[rows, :], out_hbm.at[rows, :], out_sem.at[i])

    def step_rows(s):
        return pl.ds(pl.multiple_of((s & 3) * _STEP_ROWS, _STEP_ROWS), _STEP_ROWS)

    def q_piece(s, i):
        cols = pl.ds(pl.multiple_of(i * _DH, _DH), _DH)
        q = jnp.dot(x_buf[step_rows(s), :], wq_buf[s >> 2, :, cols], preferred_element_type=jnp.float32)
        q = (q * _QSCALE).astype(jnp.bfloat16)
        q_s[s & (_NQ - 1), i] = q
        return q

    def o_piece(t, i):
        rows = pl.ds(pl.multiple_of((t & 7) * _HALF_ROWS, _HALF_ROWS), _HALF_ROWS)
        cols = pl.ds(pl.multiple_of(i * (_D // 4), _D // 4), _D // 4)
        o = jnp.concatenate([o_s[t & 1, j] for j in range(_REP)], axis=1)
        y = jnp.dot(o, wo_buf[t >> 3, :, cols], preferred_element_type=jnp.float32)
        a = acc[rows, cols] + y
        acc[rows, cols] = a
        out_buf[rows, cols] = a.astype(jnp.bfloat16)
        return y

    def scores(u):
        s = u >> 3
        rows = pl.ds(pl.multiple_of((u & (_STEP_UNITS - 1)) * _SQ, _SQ), _SQ)
        k = k_buf[u & (_NK - 1)]
        out = []
        for t in range(2):
            heads = range(t * _REP // 2, (t + 1) * _REP // 2)
            q = jnp.concatenate([q_s[s & (_NQ - 1), j, rows, :] for j in heads], axis=0)
            out.append(jax.lax.dot_general(q, k, _NT, preferred_element_type=jnp.float32))
        return out

    def softmax(sc):
        m = jnp.max(sc, axis=1, keepdims=True)
        p = jnp.exp2(sc - m)
        return p.astype(jnp.bfloat16), jnp.sum(p, axis=1, keepdims=True)

    def attend(u, t, p, l):
        rows = pl.ds(pl.multiple_of((u & 3) * _SQ, _SQ), _SQ)
        o = jnp.dot(p, v_buf[u & (_NV - 1)], preferred_element_type=jnp.float32)
        o = (o * (1.0 / l)).astype(jnp.bfloat16)
        for j in range(_REP // 2):
            o_s[(u >> 2) & 1, t * (_REP // 2) + j, rows, :] = o[j * _SQ:(j + 1) * _SQ, :]
        return o

    def await_weights(u):
        g = u >> 5

        @pl.when((u & (_B - 1)) == 4)
        def _():
            wo_cp(g).wait()

        @pl.when(jnp.logical_and((u & (_B - 1)) == _STEP_UNITS, g < _HKV - 1))
        def _():
            wq_cp(g + 1).wait()

    def make_unit(at, *, do_q, do_o, do_w=False, last_phase=False, split=False):
        names = [name for name, _ in at]
        assert sum(r for _, r in at) == _SK

        def unit(u, carry):
            n = u + _LK
            seen = []

            def request(name, val=None):
                if name in names:
                    g = names.index(name)
                    r0, nr = sum(r for _, r in at[:g]), at[g][1]
                    seen.append(name)
                    if val is not None:
                        k_buf[_NK, pl.ds(0, _SQ), :] = val[:_SQ, :_DH].astype(jnp.bfloat16)
                    if last_phase:
                        pl.when(n < _U_INORDER)(lambda: k_piece(n, r0, nr).start(priority=0))
                    else:
                        k_piece(n, r0, nr).start(priority=0)
                if do_w and name in (_AT_WO, _AT_WQ):
                    h = u >> 5
                    j = u & (_B - 1)
                    if name == _AT_WO:
                        wo_buf[_HKV, pl.ds(0, _SQ), pl.ds(0, _DH)] = val[:_SQ, :_DH].astype(jnp.bfloat16)
                        pl.when(jnp.logical_and(h < _HKV - 1, j < _GW // _WP_ROWS))(
                            lambda: wo_piece(h + 1, j).start(priority=1))
                    else:
                        wq_buf[_HKV, pl.ds(0, _SQ), pl.ds(0, _DH)] = val[:_SQ, :_DH].astype(jnp.bfloat16)
                        pl.when(jnp.logical_and(h < _HKV - 2, j < _D // _WP_ROWS))(
                            lambda: wq_piece(h + 2, j).start(priority=1))

            if do_o:
                pl.when((u & 3) == 0)(lambda: await_weights(u))
            k_cp(u).wait()
            if not split:
                for j in range(len(_VP_ROWS)):
                    v_part(u, j).wait()
                    request(f"v{j}")
            if last_phase:
                pl.when(jnp.logical_and(u + _LV >= _U_INORDER, u + _LV < _NUNITS))(
                    lambda: k_cp(u + _LV).start(priority=1))
            request("top")
            if split:
                request("y", o_piece((u >> 2) - 1, u & 3))
            sa, sb = scores(u)
            request("sA7", sa[:, 7 * _DH:])
            request("sA15", sa[:, 15 * _DH:])
            request("sB7", sb[:, 7 * _DH:])
            request("sB15", sb[:, 15 * _DH:])
            pa, la = softmax(sa)
            if split:
                for j in range(len(_VP_ROWS)):
                    v_part(u, j).wait()
                pl.when(u == _NUNITS - 1)(lambda: out_cp(0, _EARLY_ROWS, 0).start())
            request("mid")
            pb, lb = softmax(sb)
            request("pB7", pb[:, 7 * _DH:])
            request("oA", attend(u, 0, pa, la))
            request("oB", attend(u, 1, pb, lb))
            if do_o and not split:
                request("y", o_piece((u >> 2) - 1, u & 3))
            if do_q:
                request("q", q_piece((u >> 3) + _QA, u & (_STEP_UNITS - 1)))
            if last_phase:
                pl.when(u + _LV < _NUNITS)(lambda: v_start(u + _LV))
            else:
                v_start(u + _LV)
            assert sorted(seen) == sorted(names), (seen, names)
            return carry

        return unit

    def x_piece(j):
        rows = pl.ds(pl.multiple_of(j * (_ROWS // _NP0), _ROWS // _NP0), _ROWS // _NP0)
        return pltpu.make_async_copy(x_hbm.at[rows, :], x_buf.at[rows, :], x_sem.at[0])

    def wq0_piece(j):
        rows = pl.ds(pl.multiple_of(j * (_D // _NP0), _D // _NP0), _D // _NP0)
        return pltpu.make_async_copy(wq_hbm.at[rows, pl.ds(0, _GW)], wq_buf.at[0, rows], wq0_sem.at[j])

    def first_k_piece(p):
        n = p >> 3
        rows = pl.ds(pl.multiple_of((p & (_KP0 - 1)) * _KP0_ROWS, _KP0_ROWS), _KP0_ROWS)
        return pltpu.make_async_copy(k_hbm.at[n, 0, rows], k_buf.at[n, rows], k_sem.at[n])

    x_piece(0).start(priority=0)

    def first_wq(j, carry):
        wq0_piece(j).start(priority=1)
        return carry

    jax.lax.fori_loop(0, _NP0, first_wq, 0)

    def first_low(j, carry):
        n_v = 0
        for jj, what in enumerate(_FIRST_REQUESTS):
            if what == "V":
                pl.when(j == jj)(lambda n_v=n_v: v_start(n_v))
                n_v += 1
            elif what == "q":
                pl.when(j == jj)(lambda: wq_cp(1).start(priority=1))
            else:
                pl.when(j == jj)(lambda: wo_cp(0).start(priority=1))
        return carry

    jax.lax.fori_loop(0, len(_FIRST_REQUESTS), first_low, 0)
    acc[...] = jnp.zeros_like(acc)

    def first_x(j, carry):
        wq0_piece(j).wait()
        pl.when(j + 1 < _NP0)(lambda: x_piece(j + 1).start(priority=0))
        return carry

    jax.lax.fori_loop(0, _NP0, first_x, 0)
    x_cp().wait()

    def first_q(t, carry):
        s = t >> 1
        cols = pl.ds(pl.multiple_of((t & 1) * (_GW // 2), _GW // 2), _GW // 2)
        first_k_piece(3 * t).start(priority=0)
        q = jnp.dot(x_buf[step_rows(s), :], wq_buf[0, :, cols], preferred_element_type=jnp.float32)
        q = (q * _QSCALE).astype(jnp.bfloat16)
        for i, j in ((1, 1), (2, 3)):
            k_buf[_NK, pl.ds(0, _SQ), :] = q[:_SQ, j * _DH:(j + 1) * _DH]
            pl.when(3 * t + i < _LK * _KP0)(lambda i=i: first_k_piece(3 * t + i).start(priority=0))
        for j in range(_REP // 2):
            q_s[s, (t & 1) * (_REP // 2) + j] = q[:, j * _DH:(j + 1) * _DH]
        return carry

    assert 3 * (2 * _QA - 1) < _LK * _KP0 <= 3 * 2 * _QA
    jax.lax.fori_loop(0, 2 * _QA, first_q, 0)

    u_noq = (_NSTEPS - _QA) * _STEP_UNITS
    assert _FIRST_REQUESTS.count("V") == _LV and u_noq + _LV <= _U_INORDER <= _U_SPLIT + _LK
    jax.lax.fori_loop(0, 4, make_unit(_AT_FIRST, do_q=True, do_o=False, do_w=True), 0)
    jax.lax.fori_loop(4, u_noq, make_unit(_AT_MAIN, do_q=True, do_o=True, do_w=True), 0)
    jax.lax.fori_loop(u_noq, _U_SPLIT, make_unit(_AT_NOQ, do_q=False, do_o=True, last_phase=True), 0)
    jax.lax.fori_loop(
        _U_SPLIT, _NUNITS, make_unit(_AT_SPLIT, do_q=False, do_o=True, last_phase=True, split=True), 0)

    o = jnp.concatenate([o_s[1, j] for j in range(_REP)], axis=1)
    y = jnp.dot(o, wo_buf[_HKV - 1], preferred_element_type=jnp.float32)
    last = pl.ds(_EARLY_ROWS, _HALF_ROWS)
    out_buf[last, :] = (acc[last, :] + y).astype(jnp.bfloat16)
    out_cp(_EARLY_ROWS, _HALF_ROWS, 1).start()
    out_cp(0, _EARLY_ROWS, 0).wait()
    out_cp(_EARLY_ROWS, _HALF_ROWS, 1).wait()


@jax.jit
def pallas_standalone__gqa_block_cached__sampling_kernel(
    x: jax.Array,
    k_cache: jax.Array,
    v_cache: jax.Array,
    wq: jax.Array,
    wo: jax.Array,
):
    assert x.shape == (_B, _SQ, _D) and k_cache.shape == v_cache.shape == (_B, _HKV, _SK, _DH)
    assert wq.shape == (_D, _HQ * _DH) and wo.shape == (_HQ * _DH, _D)
    bf16 = jnp.bfloat16
    out = pl.pallas_call(
        _kernel,
        out_shape=jax.ShapeDtypeStruct((_ROWS, _D), bf16),
        in_specs=[pl.BlockSpec(memory_space=pl.ANY)] * 5,
        out_specs=pl.BlockSpec(memory_space=pl.ANY),
        scratch_shapes=[
            pltpu.VMEM((_ROWS, _D), bf16),
            pltpu.VMEM((_HKV + 1, _D, _GW), bf16),
            pltpu.VMEM((_HKV + 1, _GW, _D), bf16),
            pltpu.VMEM((_NK + 1, _SK, _DH), bf16),
            pltpu.VMEM((_NV, _SK, _DH), bf16),
            pltpu.VMEM((_NQ, _REP, _STEP_ROWS, _DH), bf16),
            pltpu.VMEM((2, _REP, _HALF_ROWS, _DH), bf16),
            pltpu.VMEM((_ROWS, _D), jnp.float32),
            pltpu.VMEM((_ROWS, _D), bf16),
            pltpu.SemaphoreType.DMA((1,)),
            pltpu.SemaphoreType.DMA((_HKV,)),
            pltpu.SemaphoreType.DMA((_HKV,)),
            pltpu.SemaphoreType.DMA((_NK,)),
            pltpu.SemaphoreType.DMA((_NV, len(_VP_ROWS))),
            pltpu.SemaphoreType.DMA((2,)),
            pltpu.SemaphoreType.DMA((_NP0,)),
        ],
        compiler_params=pltpu.CompilerParams(
            vmem_limit_bytes=100 * 1024 * 1024,
            disable_semaphore_checks=True,
        ),
    )(x.reshape(_ROWS, _D).astype(bf16), k_cache.astype(bf16), v_cache.astype(bf16),
      wq.astype(bf16), wo.astype(bf16))
    return out.reshape(_B, _SQ, _D).astype(x.dtype)
```
